```python
import os as _os
_os.environ.setdefault("JAX_PLATFORMS", "cpu")
import jax
import jax.numpy as jnp

def _softmax(x, axis=-1):
    return jax.nn.softmax(x, axis=axis)
def _gelu(x):
    return jax.nn.gelu(x, approximate=True)
def _silu(x):
    return jax.nn.silu(x)
def _sigmoid(x):
    return jax.nn.sigmoid(x)
def _layernorm(x, axis=-1, eps=1e-5):
    m = jnp.mean(x, axis=axis, keepdims=True)
    v = jnp.var(x, axis=axis, keepdims=True)
    return (x - m) / jnp.sqrt(v + eps)
def _scatter_add(tgt, idx, src, axis=0):
    return tgt.at[idx].add(src)
def _segment_sum(src, seg, n):
    return jax.ops.segment_sum(src, seg, n)
class _Rng:
    def __init__(self, key):
        self._k = key
    def _next(self):
        self._k, sub = jax.random.split(self._k)
        return sub
    def normal(self, shape):
        return jax.random.normal(self._next(), shape, dtype=jnp.bfloat16)
    def randint(self, lo, hi, shape):
        return jax.random.randint(self._next(), shape, lo, hi, dtype=jnp.int32)
    def uniform(self, shape, lo=0.0, hi=1.0):
        return jax.random.uniform(self._next(), shape, jnp.bfloat16, lo, hi)
    def permutation(self, n):
        return jax.random.permutation(self._next(), n)


kernel_name = 'interleave_layers__gqa_block_cached__dense_activation_silu__decode'

def setup_inputs():
    _rng = _Rng(jax.random.key(int.from_bytes(__import__("os").urandom(4), "little")))
    _w = (lambda a: (lambda t: t.astype(jnp.bfloat16) if jnp.issubdtype(t.dtype, jnp.floating) else t)(jnp.asarray(a)))
    def _A_setup():
        B, Sq, D = 2, 1, 512
        Hq, Hkv, Sk, Dh = 32, 8, 8192, 128
        assert Hq % Hkv == 0, (Hq, Hkv)
        return {
            "x": _w((lambda *s: _rng.normal(s) * 0.1)(B, Sq, D)),
            "k_cache": _w((lambda *s: _rng.normal(s) * 0.8)(B, Hkv, Sk, Dh)),
            "v_cache": _w((lambda *s: _rng.normal(s) * 1.6)(B, Hkv, Sk, Dh)),
            "wq": _w((lambda *s: _rng.normal(s) * 0.8)(D, Hq * Dh) * (D ** -0.5)),
            "wo": _w((lambda *s: _rng.normal(s) * 1.6)(Hq * Dh, D) * ((Hq * Dh) ** -0.5)),
        }
    _A_in = _A_setup()

    def _B_setup():
        B, S, D, F = 2, 1, 512, 1792
        return {
            "x": _w((lambda *s: _rng.normal(s) * 0.1)(B, S, D)),
            "w1": _w((lambda *s: _rng.normal(s) * 0.4)(D, F) * (D ** -0.5)),
            "w2": _w((lambda *s: _rng.normal(s) * 0.4)(F, D) * (F ** -0.5)),
        }
    _B_in = _B_setup()

    return {
        "A_x": _A_in["x"],
        "A_k_cache": _A_in["k_cache"],
        "A_v_cache": _A_in["v_cache"],
        "A_wq": _A_in["wq"],
        "A_wo": _A_in["wo"],
        "B_x": _B_in["x"],
        "B_w1": _B_in["w1"],
        "B_w2": _B_in["w2"],
    }

def reference(A_x, A_k_cache, A_v_cache, A_wq, A_wo, B_x, B_w1, B_w2):
    def _A_ref(x, k_cache, v_cache, wq, wo):
        B, Sq, D = x.shape
        Hq, Dh = 32, 128
        Hkv = k_cache.shape[1]
        rep = Hq // Hkv
        q = (lambda x, *d: x.transpose(*d))((x @ wq).reshape(B, Sq, Hq, Dh), 0, 2, 1, 3)
        k = jnp.repeat(k_cache, rep, axis=1)
        v = jnp.repeat(v_cache, rep, axis=1)
        scores = jnp.einsum("bhqd,bhkd->bhqk", q, k) * (Dh ** -0.5)
        p = _softmax(scores, axis=-1)
        o = jnp.einsum("bhqk,bhkd->bhqd", p, v)
        return (lambda x, *d: x.transpose(*d))(o, 0, 2, 1, 3).reshape(B, Sq, Hq * Dh) @ wo

    def _B_ref(x, w1, w2):
        h = jnp.einsum("bsd,df->bsf", x, w1)
        h = _silu(h)
        out = jnp.einsum("bsf,fd->bsd", h, w2)
        return out

    x = A_x
    x = x + _A_ref(_layernorm(x, axis=-1), A_k_cache, A_v_cache, A_wq, A_wo)
    x = x + _B_ref(_layernorm(x, axis=-1), B_w1, B_w2)
    x = x + _A_ref(_layernorm(x, axis=-1), A_k_cache, A_v_cache, A_wq, A_wo)
    x = x + _B_ref(_layernorm(x, axis=-1), B_w1, B_w2)
    return x
```

```python
import functools
import jax
import jax.numpy as jnp
import jax.experimental.pallas as pl
import jax.experimental.pallas.tpu as pltpu

B, D = 2, 512
HQ, HKV, SK, DH = 32, 8, 8192, 128
REP = HQ // HKV
F = 1792
NG = 4
QK = SK // NG
EPS = 1e-5
SCALE = DH ** -0.5
PAD = 128
VSPLIT = 4

f32 = jnp.float32
bf16 = jnp.bfloat16


def _mo(i, n):
    return i if isinstance(i, int) else pl.multiple_of(i, n)


def _dot(a, b):
    return jnp.dot(a, b, preferred_element_type=f32)


def _dot_nt(a, b):
    return jax.lax.dot_general(a, b, (((1,), (1,)), ((), ())), preferred_element_type=f32)


def _kernel(x_hbm, k_hbm, v_hbm, wq_hbm, wo_hbm, w1_hbm, w2_hbm, o_ref,
            xbuf, kbuf, vbuf, ktbuf, wq, wo, w1, w2, qs, ksem, vsem, wsem, lsem):
    def kcp(b, h):
        return pltpu.make_async_copy(k_hbm.at[b, h], kbuf.at[b, h], ksem.at[b * HKV + h])

    def vcp(b, h):
        return pltpu.make_async_copy(v_hbm.at[b, h], vbuf.at[b, h], vsem.at[b * HKV + h])

    def vlast(g):
        return pltpu.make_async_copy(v_hbm.at[1, HKV - 1, pl.ds(_mo(g * QK, QK), QK)],
                                     vbuf.at[1, HKV - 1, pl.ds(_mo(g * QK, QK), QK)], lsem.at[g])

    xcp = pltpu.make_async_copy(x_hbm, xbuf, wsem.at[0])
    wqcp = pltpu.make_async_copy(wq_hbm, wq.at[:, pl.ds(0, HQ * DH)], wsem.at[1])
    wocp = pltpu.make_async_copy(wo_hbm, wo.at[:, pl.ds(0, D)], wsem.at[2])
    w1cp = pltpu.make_async_copy(w1_hbm, w1, wsem.at[3])
    w2cp = pltpu.make_async_copy(w2_hbm, w2.at[:, pl.ds(0, D)], wsem.at[4])

    xcp.start()
    wqcp.start()

    def issue(i, c):
        b = i // HKV
        h = i % HKV
        kcp(b, h).start()

        @pl.when(i < B * HKV - 1)
        def _():
            vcp(b, h).start()

        @pl.when(i == HKV - 1)
        def _():
            wocp.start()
            w1cp.start()
            w2cp.start()
        return c

    jax.lax.fori_loop(0, B * HKV, issue, 0)

    def issue_last(g, c):
        vlast(g).start()
        return c

    jax.lax.fori_loop(0, NG, issue_last, 0)

    row16 = jax.lax.broadcasted_iota(jnp.int32, (16, DH), 0)
    r16_mod = row16 % REP
    r16_div = row16 // REP

    def center(x):
        m = jnp.mean(x, axis=-1, keepdims=True)
        xc = x - m
        var = jnp.mean(xc * xc, axis=-1, keepdims=True)
        rstd = jax.lax.rsqrt(var + EPS)
        return xc.astype(bf16), rstd

    def make_q(x):
        xc, rstd = center(x)
        q = _dot(xc, wq[:, 0:HQ * DH]) * (rstd * SCALE)
        for h in range(HKV):
            t = q[:, (REP * h) * DH:(REP * h + 1) * DH]
            for i in range(1, REP):
                t = jnp.where(r16_mod == i, q[:, (REP * h + i) * DH:(REP * h + i + 1) * DH], t)
            blocks = [jnp.where(r16_div == g, t, 0.0).astype(bf16) for g in range(NG)]
            qs[h] = jnp.concatenate(blocks, axis=1)

    def softmax_p(s):
        m = jnp.max(s, axis=-1, keepdims=True)
        mb = jnp.broadcast_to(m, (16, DH))
        mb = jnp.maximum(mb, pltpu.roll(mb, 8, 0))
        mb = jnp.maximum(mb, pltpu.roll(mb, 4, 0))
        p = jnp.exp(s - mb[:, :1])
        l = jnp.sum(p, axis=-1, keepdims=True)
        lb = jnp.broadcast_to(l, (16, DH))
        lb = lb + pltpu.roll(lb, 8, 0)
        lb = lb + pltpu.roll(lb, 4, 0)
        return p.astype(bf16), lb

    def finish_head(rs, lb, h):
        o = rs[0]
        for g in range(1, NG):
            o = jnp.where(r16_div == g, rs[g], o)
        o = o / lb
        ocat = jnp.concatenate([jnp.where(r16_mod == i, o, 0.0).astype(bf16) for i in range(REP)], axis=1)
        start = h * (REP * DH)
        if not isinstance(h, int):
            start = pl.multiple_of(start, REP * DH)
        return _dot(ocat, wo[pl.ds(start, REP * DH), 0:D])

    def pv(p, b, h):
        return [_dot(p, vbuf[b, h, pl.ds(g * QK, QK), :]) for g in range(NG)]

    def ffn(x):
        xc, rstd = center(x)
        hh = _dot(xc, w1[...]) * rstd
        hh = hh * jax.nn.sigmoid(hh)
        return x + _dot(hh.astype(bf16), w2[:, 0:D])

    def resid(x, y):
        return x + jnp.sum(y, axis=0, keepdims=True)

    def s_xpose(b, h):
        qh = qs[h]
        s = None
        for g in range(NG):
            t = _dot_nt(qh[:, g * DH:(g + 1) * DH], kbuf[b, h, pl.ds(g * QK, QK), :])
            s = t if s is None else s + t
        return s

    xcp.wait()
    wqcp.wait()

    xin = xbuf[...].astype(f32)
    x0 = jnp.broadcast_to(xin[0:1, :], (16, D))
    make_q(x0)

    obuf0 = jnp.zeros((HKV, 16, DH), f32)

    def body00(h, carry):
        kcp(0, h).wait()
        s = s_xpose(0, h)
        p, lb = softmax_p(s)
        vcp(0, h).wait()
        rs = pv(p, 0, h)
        o = rs[0]
        for g in range(1, NG):
            o = jnp.where(r16_div == g, rs[g], o)
        o = o / lb
        ocat = jnp.concatenate([jnp.where(r16_mod == i, o, 0.0).astype(bf16) for i in range(REP)], axis=1)
        qs[h] = ocat
        return carry

    jax.lax.fori_loop(0, HKV, body00, 0)
    wocp.wait()
    y = None
    for h in range(HKV):
        t = _dot(qs[h], wo[h * 512:(h + 1) * 512, 0:D])
        y = t if y is None else y + t
    x0 = resid(x0, y)
    w1cp.wait()
    w2cp.wait()
    x0 = ffn(x0)
    make_q(x0)

    def body01(h, y):
        s = s_xpose(0, h)
        p, lb = softmax_p(s)
        rs = pv(p, 0, h)
        return y + finish_head(rs, lb, h)

    y = jax.lax.fori_loop(0, HKV, body01, jnp.zeros((16, D), f32))
    x0 = resid(x0, y)
    x0 = ffn(x0)

    x1 = jnp.broadcast_to(xin[1:2, :], (16, D))
    make_q(x1)
    eye = (jax.lax.broadcasted_iota(jnp.int32, (DH, DH), 0)
           == jax.lax.broadcasted_iota(jnp.int32, (DH, DH), 1)).astype(bf16)

    def s_xpose_t(h):
        qh = qs[h]
        s = None
        for g in range(NG):
            lhs = jnp.concatenate([qh[:, g * DH:(g + 1) * DH], eye], axis=0)
            t = _dot_nt(lhs, kbuf[1, h, pl.ds(g * QK, QK), :])
            ktbuf[h, pl.ds(g * DH, DH), 0:QK] = t[16:].astype(bf16)
            s = t[:16] if s is None else s + t[:16]
        return s

    def body10(h, y):
        kcp(1, h).wait()
        s = s_xpose_t(h)
        p, lb = softmax_p(s)
        vcp(1, h).wait()
        rs = pv(p, 1, h)
        return y + finish_head(rs, lb, h)

    y = jax.lax.fori_loop(0, HKV - 1, body10, jnp.zeros((16, D), f32))
    h = HKV - 1
    kcp(1, h).wait()
    s = s_xpose_t(h)
    p, lb = softmax_p(s)
    rs = []
    for g in range(NG):
        vlast(g).wait()
        rs.append(_dot(p, vbuf[1, h, pl.ds(g * QK, QK), :]))
    y = y + finish_head(rs, lb, h)
    x1 = resid(x1, y)
    x1 = ffn(x1)
    make_q(x1)
    y = None
    s_next = _dot(qs[0], ktbuf[0, :, 0:QK])
    for h in range(HKV):
        s = s_next
        if h + 1 < HKV:
            s_next = _dot(qs[h + 1], ktbuf[h + 1, :, 0:QK])
        p, lb = softmax_p(s)
        rs = pv(p, 1, h)
        t = finish_head(rs, lb, h)
        y = t if y is None else y + t
    x1 = resid(x1, y)
    x1 = ffn(x1)
    row2 = jax.lax.broadcasted_iota(jnp.int32, (2, D), 0)
    o_ref[...] = jnp.where(row2 == 0, x0[0:2, :], x1[0:2, :]).astype(o_ref.dtype)


@jax.jit
def pallas_interleave_layers__gqa_block_cached__dense_activation_silu__decode_kernel(
    A_x, A_k_cache, A_v_cache, A_wq, A_wo, B_x, B_w1, B_w2,
):
    del B_x
    any_spec = pl.BlockSpec(memory_space=pl.ANY)
    return pl.pallas_call(
        _kernel,
        out_shape=jax.ShapeDtypeStruct((B, D), A_x.dtype),
        in_specs=[any_spec] * 7,
        out_specs=pl.BlockSpec(memory_space=pltpu.VMEM),
        scratch_shapes=[
            pltpu.VMEM((B, D), bf16),
            pltpu.VMEM((B, HKV, SK, DH), bf16),
            pltpu.VMEM((B, HKV, SK, DH), bf16),
            pltpu.VMEM((HKV, NG * DH, QK + PAD), bf16),
            pltpu.VMEM((D, HQ * DH + PAD), bf16),
            pltpu.VMEM((HQ * DH, D + PAD), bf16),
            pltpu.VMEM((D, F), bf16),
            pltpu.VMEM((F, D + PAD), bf16),
            pltpu.VMEM((HKV, 16, NG * DH), bf16),
            pltpu.SemaphoreType.DMA((B * HKV,)),
            pltpu.SemaphoreType.DMA((B * HKV,)),
            pltpu.SemaphoreType.DMA((5,)),
            pltpu.SemaphoreType.DMA((NG,)),
        ],
        compiler_params=pltpu.CompilerParams(vmem_limit_bytes=110 * 1024 * 1024, disable_semaphore_checks=True),
    )(A_x.reshape(B, D), A_k_cache, A_v_cache, A_wq, A_wo, B_w1, B_w2).reshape(A_x.shape)
```

```python
import functools
import jax
import jax.numpy as jnp
import jax.experimental.pallas as pl
import jax.experimental.pallas.tpu as pltpu

B, D = 2, 512
HQ, HKV, SK, DH = 32, 8, 8192, 128
REP = HQ // HKV
F = 1792
NG = 4
QK = SK // NG
EPS = 1e-5
SCALE = DH ** -0.5
PAD = 128
T = 128
ND = D // T
NF = F // T
HW = REP * DH
NVQ = 6
NVO = 6
LOG2E = 1.4426950408889634

f32 = jnp.float32
bf16 = jnp.bfloat16
u32 = jnp.uint32


def _mo(i, n):
    return i if isinstance(i, int) else pl.multiple_of(i, n)


def _dot(a, b):
    return jnp.dot(a, b, preferred_element_type=f32)


def _dot_nt(a, b):
    return jax.lax.dot_general(a, b, (((1,), (1,)), ((), ())), preferred_element_type=f32)


def _fold(r):
    return r[0:8] + r[8:16]


def _hilo(x):
    hi = x.astype(bf16)
    lo = (x - hi.astype(f32)).astype(bf16)
    return jnp.concatenate([hi, lo], axis=0)


def _rowsum(y):
    y = y + pltpu.roll(y, 4, 0)
    y = y + pltpu.roll(y, 2, 0)
    y = y + pltpu.roll(y, 1, 0)
    return y


def _kernel(x_hbm, k_hbm, v_hbm, wq_hbm, wo_hbm, w1_hbm, w2_hbm, o_ref,
            xbuf, k1buf, v1buf, wq, wo, w1, w2, qs, csq, cs1, xb, x0out, zsm,
            ksem, vsem, wsem, lsem):
    def k1cp(h):
        return pltpu.make_async_copy(k_hbm.at[1, h], k1buf.at[h], ksem.at[HKV + h])

    def v1cp(h):
        return pltpu.make_async_copy(v_hbm.at[1, h], v1buf.at[h], vsem.at[HKV + h])

    def vlast(g):
        return pltpu.make_async_copy(v_hbm.at[1, HKV - 1, pl.ds(_mo(g * QK, QK), QK)],
                                     v1buf.at[HKV - 1, pl.ds(_mo(g * QK, QK), QK)], lsem.at[g])

    xcp = pltpu.make_async_copy(x_hbm, xbuf, wsem.at[0])
    wqcp = pltpu.make_async_copy(wq_hbm, wq.at[:, pl.ds(0, HQ * DH)], wsem.at[1])
    wocp = pltpu.make_async_copy(wo_hbm, wo.at[:, pl.ds(0, D)], wsem.at[2])
    w1cp = pltpu.make_async_copy(w1_hbm, w1, wsem.at[3])
    w2cp = pltpu.make_async_copy(w2_hbm, w2.at[:, pl.ds(0, D)], wsem.at[4])

    row8 = jax.lax.broadcasted_iota(jnp.int32, (8, T), 0)
    r8_mod = row8 % REP
    r8_lo = row8 < REP
    zero8 = jnp.zeros((8, T), f32)

    def stats(xt):
        s = (xt[0] + xt[1]) + (xt[2] + xt[3])
        m = jnp.sum(s, axis=-1, keepdims=True) * (1.0 / D)
        c = [t - m for t in xt]
        v = (c[0] * c[0] + c[1] * c[1]) + (c[2] * c[2] + c[3] * c[3])
        var = jnp.sum(v, axis=-1, keepdims=True) * (1.0 / D)
        return m, jax.lax.rsqrt(var + EPS)

    def q_head(q, h):
        t = q[:, 0:DH]
        for i in range(1, REP):
            t = jnp.where(r8_mod == i, q[:, i * DH:(i + 1) * DH], t)
        a = jnp.where(r8_lo, t, 0.0)
        b = jnp.where(r8_lo, 0.0, t)
        blocks = [jnp.concatenate(p, axis=0).astype(bf16)
                  for p in ((a, zero8), (b, zero8), (zero8, a), (zero8, b))]
        qs[h] = jnp.concatenate(blocks, axis=1)

    def make_q(xt):
        lc = jnp.concatenate([_hilo(t) for t in xt], axis=1)
        m, rstd = stats(xt)
        sc = rstd * SCALE
        for h in range(HKV):
            r = _fold(_dot(lc, wq[:, h * HW:(h + 1) * HW]))
            q_head((r - m * csq[:, h * HW:(h + 1) * HW]) * sc, h)

    def softmax_p(s, sc=None):
        mx = jnp.maximum(s[0:8], s[8:16])
        m = jnp.max(mx, axis=-1, keepdims=True)
        mb = jnp.broadcast_to(m, (8, T))
        mb = jnp.maximum(mb, pltpu.roll(mb, 4, 0))
        mb = jnp.concatenate([mb, mb], axis=0)
        if sc is None:
            p = jnp.exp(s - mb[:, :1])
        else:
            p = jnp.exp2((s - mb[:, :1]) * sc)
        l = jnp.sum(p[0:8] + p[8:16], axis=-1, keepdims=True)
        lb = jnp.broadcast_to(l, (8, T))
        lb = lb + pltpu.roll(lb, 4, 0)
        return p.astype(bf16), lb

    def make_ocat(rs, lb):
        o = jnp.where(r8_lo, rs[0][0:8], rs[1][0:8]) + jnp.where(r8_lo, rs[2][8:16], rs[3][8:16])
        o = o / lb
        return jnp.concatenate([_hilo(jnp.where(r8_mod == i, o, 0.0)) for i in range(REP)], axis=1)

    def wo_head(ocat, h):
        return _fold(_dot(ocat, wo[pl.ds(_mo(h * HW, HW), HW), 0:D]))

    def wo_last(xt, y, ocat, h):
        out = []
        for n in range(ND):
            t = _fold(_dot(ocat, wo[h * HW:(h + 1) * HW, n * T:(n + 1) * T]))
            if y is not None:
                t = t + y[:, n * T:(n + 1) * T]
            out.append(xt[n] + _rowsum(t))
        return out

    def ffn(xt, ksplit):
        lhs = [_hilo(t) for t in xt]
        m, rstd = stats(xt)
        acc = None
        for k in range(ND):
            t = _fold(_dot(lhs[k], w1[k * T:(k + 1) * T, :]))
            acc = t if acc is None else acc + t
        hh = (acc - m * cs1[...]) * rstd
        hh = hh * jax.nn.sigmoid(hh)
        hl = _hilo(hh)
        acc = None
        for k in range(ksplit):
            t = _fold(_dot(hl[:, k * T:(k + 1) * T], w2[k * T:(k + 1) * T, 0:D]))
            acc = t if acc is None else acc + t
        out = []
        for n in range(ND):
            t = acc[:, n * T:(n + 1) * T]
            if ksplit < NF:
                t = t + _fold(_dot(hl[:, ksplit * T:], w2[ksplit * T:, n * T:(n + 1) * T]))
            out.append(xt[n] + t)
        return out

    def load_x(b):
        xin = xbuf[...].astype(f32)
        return [jnp.broadcast_to(xin[b:b + 1, n * T:(n + 1) * T], (8, T)) for n in range(ND)]

    def batch0(k0buf, v0buf):
        def k0cp(h):
            return pltpu.make_async_copy(k_hbm.at[0, h], k0buf.at[h], ksem.at[h])

        def v0cp(h):
            return pltpu.make_async_copy(v_hbm.at[0, h], v0buf.at[h], vsem.at[h])

        xcp.start()
        wqcp.start()

        def issue0(h, c):
            k0cp(h).start()
            v0cp(h).start()
            return c

        jax.lax.fori_loop(0, HKV, issue0, 0)
        wocp.start()
        w1cp.start()
        w2cp.start()

        def issue1(h, c):
            k1cp(h).start()

            @pl.when(h < HKV - 1)
            def _():
                v1cp(h).start()
            return c

        jax.lax.fori_loop(0, HKV, issue1, 0)

        def issue_last(g, c):
            vlast(g).start()
            zsm[0] = g // NG
            return c

        jax.lax.fori_loop(0, NG, issue_last, 0)

        def s_xpose(h):
            qh = qs[h]
            s = None
            for g in range(NG):
                t = _dot_nt(qh[:, g * DH:(g + 1) * DH], k0buf[h, pl.ds(g * QK, QK), :])
                s = t if s is None else s + t
            return s

        def pv0(p, h):
            return [_dot(p, v0buf[h, pl.ds(g * QK, QK), :]) for g in range(NG)]

        xcp.wait()
        wqcp.wait()
        ones16 = jnp.ones((16, D), bf16)
        csq[...] = _dot(ones16, wq[:, 0:HQ * DH])[0:8]
        x0 = load_x(0)
        make_q(x0)

        def body00(h, carry):
            k0cp(h).wait()
            p, lb = softmax_p(s_xpose(h))
            v0cp(h).wait()
            qs[h] = make_ocat(pv0(p, h), lb)
            return carry

        jax.lax.fori_loop(0, HKV, body00, 0)
        wocp.wait()
        y = None
        for h in range(HKV - 1):
            t = wo_head(qs[h], h)
            y = t if y is None else y + t
        x0 = wo_last(x0, y, qs[HKV - 1], HKV - 1)
        w1cp.wait()
        w2cp.wait()
        cs1[...] = _dot(ones16, w1[...])[0:8]
        x0 = ffn(x0, NF)
        make_q(x0)

        def body01(h, y):
            p, lb = softmax_p(s_xpose(h))
            return y + wo_head(make_ocat(pv0(p, h), lb), h)

        y = jax.lax.fori_loop(0, HKV, body01, jnp.zeros((8, D), f32))
        y = _rowsum(y)
        x0 = [x0[n] + y[:, n * T:(n + 1) * T] for n in range(ND)]
        x0 = ffn(x0, NF)
        x0out[...] = jnp.concatenate(x0, axis=1)

    pl.run_scoped(batch0, pltpu.VMEM((HKV, SK, DH), bf16), pltpu.VMEM((HKV, SK, DH), bf16))

    def batch1(ktu, v1u, wqf, wof):
        def cvt(j, c):
            r = pl.ds(pl.multiple_of(j * 64, 64), 64)
            for h in range(NVQ):
                hh = HKV - NVQ + h
                wqf[h, r, :] = wq[r, hh * HW:(hh + 1) * HW].astype(f32)
            for h in range(NVO):
                wof[h, r, :] = wo[pl.ds(pl.multiple_of(h * HW + j * 64, 64), 64), 0:D].astype(f32)
            return c

        jax.lax.fori_loop(0, HW // 64, cvt, 0)

        x1 = load_x(1)
        make_q(x1)
        eye = (jax.lax.broadcasted_iota(jnp.int32, (DH, DH), 0)
               == jax.lax.broadcasted_iota(jnp.int32, (DH, DH), 1)).astype(bf16)

        def s_xpose_t(h):
            qh = qs[h]
            s = None
            for g in range(NG):
                lhs = jnp.concatenate([qh[:, g * DH:(g + 1) * DH], eye], axis=0)
                t = _dot_nt(lhs, k1buf[h, pl.ds(g * QK, QK), :])
                ktu[h, pl.ds(g * (DH // 2), DH // 2), 0:QK] = pltpu.bitcast(t[16:].astype(bf16), u32)
                s = t[:16] if s is None else s + t[:16]
            return s

        def pv_copy(p, h, g):
            v = v1buf[h, pl.ds(g * QK, QK), :]
            v1u[h, pl.ds(g * (QK // 2), QK // 2), :] = pltpu.bitcast(v, u32)
            return _dot(p, v)

        def body10(h, y):
            k1cp(h).wait()
            p, lb = softmax_p(s_xpose_t(h))
            v1cp(h).wait()
            rs = [pv_copy(p, h, g) for g in range(NG)]
            return y + wo_head(make_ocat(rs, lb), h)

        y = jax.lax.fori_loop(0, HKV - 1, body10, jnp.zeros((8, D), f32))
        h = HKV - 1
        k1cp(h).wait()
        p, lb = softmax_p(s_xpose_t(h))
        rs = []
        for g in range(NG):
            vlast(g).wait()
            rs.append(pv_copy(p, h, g))
        x1 = wo_last(x1, y, make_ocat(rs, lb), h)
        x1 = ffn(x1, 10)

        zero = zsm[0]
        zvec = jnp.full((8, T), zero, jnp.int32)
        lhs = [_hilo(t) for t in x1]
        m, rstd = stats(x1)
        sc = jnp.concatenate([rstd, rstd], axis=0) * (SCALE * LOG2E)
        acc = None
        for k in range(ND):
            t = _fold(_dot(lhs[k], wq[k * T:(k + 1) * T, 0:HW]))
            acc = t if acc is None else acc + t
        q_head(acc - m * csq[:, 0:HW], 0)
        lc = jnp.concatenate(lhs, axis=1)
        for h in range(1, HKV - NVQ):
            r = _fold(_dot(lc, wq[:, h * HW:(h + 1) * HW]))
            q_head(r - m * csq[:, h * HW:(h + 1) * HW], h)
        for n in range(ND):
            xb[pl.ds(pl.multiple_of(zero + n * T, T), T), :] = jnp.transpose(jnp.broadcast_to(x1[n][0:1, :], (T, T)))

        def vpu_matvec(colb, w_ref, j):
            accs = [None, None]
            for kg in range(HW // 8):
                c = colb(kg)
                t = w_ref[j, kg * 8:(kg + 1) * 8, :] * jnp.concatenate([c] * 4, axis=1)
                a = kg % 2
                accs[a] = t if accs[a] is None else accs[a] + t
            return accs[0] + accs[1]

        def tie(a, dep):
            z4 = jnp.concatenate([zvec] * 4, axis=1)
            bits = pltpu.bitcast(a, jnp.int32) | (pltpu.bitcast(dep, jnp.int32) & z4)
            return pltpu.bitcast(bits, f32)

        def vpu_q(h, dep):
            r = _rowsum(vpu_matvec(lambda kg: xb[kg * 8:(kg + 1) * 8, :], wqf, h - (HKV - NVQ)))
            if dep is not None:
                r = tie(r, dep)
            q_head(r - m * csq[:, h * HW:(h + 1) * HW], h)

        def vpu_o(rs, lb, h):
            o = jnp.where(r8_lo, rs[0][0:8], rs[1][0:8]) + jnp.where(r8_lo, rs[2][8:16], rs[3][8:16])
            o = (o + pltpu.roll(o, 4, 0)) / lb
            ob = [jnp.transpose(jnp.broadcast_to(o[i:i + 1, :], (T, T))) for i in range(REP)]
            return vpu_matvec(lambda kg: ob[kg // 16][(kg % 16) * 8:(kg % 16 + 1) * 8, :], wof, h)

        def qk(h):
            return _dot(qs[h], pltpu.bitcast(ktu[h, :, 0:QK], bf16))

        def pv(p, h):
            return [_dot(p, pltpu.bitcast(v1u[h, pl.ds(g * (QK // 2), QK // 2), :], bf16)) for g in range(NG)]

        y = None
        ss = {0: qk(0)}
        oc = {}
        for h in range(HKV):
            if h + 2 >= HKV - NVQ and h + 2 < HKV:
                vpu_q(h + 2, y)
            if h + 1 < HKV:
                ss[h + 1] = qk(h + 1)
            p, lb = softmax_p(ss.pop(h), sc)
            rs = pv(p, h)
            if h < NVO:
                t = vpu_o(rs, lb, h)
                y = t if y is None else y + t
            else:
                oc[h] = make_ocat(rs, lb)
            if h - 1 in oc:
                t = wo_head(oc.pop(h - 1), h - 1)
                y = t if y is None else y + t
        x1 = wo_last(x1, y, oc.pop(HKV - 1), HKV - 1)
        x1 = ffn(x1, NF)
        row2 = jax.lax.broadcasted_iota(jnp.int32, (2, D), 0)
        xo1 = jnp.concatenate(x1, axis=1)
        o_ref[...] = jnp.where(row2 == 0, x0out[0:2, :], xo1[0:2, :]).astype(o_ref.dtype)

    pl.run_scoped(batch1,
                  pltpu.VMEM((HKV, NG * DH // 2, QK + PAD), u32),
                  pltpu.VMEM((HKV, SK // 2, DH), u32),
                  pltpu.VMEM((NVQ, D, HW), f32),
                  pltpu.VMEM((NVO, HW, D), f32))


@jax.jit
def pallas_interleave_layers__gqa_block_cached__dense_activation_silu__decode_kernel(
    A_x, A_k_cache, A_v_cache, A_wq, A_wo, B_x, B_w1, B_w2,
):
    del B_x
    any_spec = pl.BlockSpec(memory_space=pl.ANY)
    return pl.pallas_call(
        _kernel,
        out_shape=jax.ShapeDtypeStruct((B, D), A_x.dtype),
        in_specs=[any_spec] * 7,
        out_specs=pl.BlockSpec(memory_space=pltpu.VMEM),
        scratch_shapes=[
            pltpu.VMEM((B, D), bf16),
            pltpu.VMEM((HKV, SK, DH), bf16),
            pltpu.VMEM((HKV, SK, DH), bf16),
            pltpu.VMEM((D, HQ * DH + PAD), bf16),
            pltpu.VMEM((HQ * DH, D + PAD), bf16),
            pltpu.VMEM((D, F), bf16),
            pltpu.VMEM((F, D + PAD), bf16),
            pltpu.VMEM((HKV, 16, NG * DH), bf16),
            pltpu.VMEM((8, HQ * DH), f32),
            pltpu.VMEM((8, F), f32),
            pltpu.VMEM((D, T), f32),
            pltpu.VMEM((8, D), f32),
            pltpu.SMEM((1,), jnp.int32),
            pltpu.SemaphoreType.DMA((B * HKV,)),
            pltpu.SemaphoreType.DMA((B * HKV,)),
            pltpu.SemaphoreType.DMA((5,)),
            pltpu.SemaphoreType.DMA((NG,)),
        ],
        compiler_params=pltpu.CompilerParams(vmem_limit_bytes=110 * 1024 * 1024, disable_semaphore_checks=True),
    )(A_x.reshape(B, D), A_k_cache, A_v_cache, A_wq, A_wo, B_w1, B_w2).reshape(A_x.shape)
```

```python
import jax
import jax.numpy as jnp
import jax.experimental.pallas as pl
import jax.experimental.pallas.tpu as pltpu

B, D = 2, 512
HQ, HKV, SK, DH = 32, 8, 8192, 128
REP = HQ // HKV
F = 1792
NG = 4
QK = SK // NG
EPS = 1e-5
SCALE = DH ** -0.5
LOG2E = 1.4426950408889634
PAD = 128
T = 128
ND = D // T
NF = F // T
NC = QK // T
HW = REP * DH

NVQ = 6
NVO = 6
FA = 4
FC = 5
FB = NF - FA - FC
NM1 = FA + FB
NM2 = FB + FC
FX = (0, 1)
FXM = max(FX)
NVC = (0, 0, 6, 6, 6, 12, 12, 12)
NVCM = max(NVC)
KG = 6
NGRP = -(-NVCM // KG)
GH0 = [min(h for h in range(HKV) if NVC[h] > g * KG) for g in range(NGRP)]
GBASE = [sum(HKV - GH0[k] for k in range(g)) for g in range(NGRP)]
NSLOT = sum(HKV - h for h in GH0)
assert all(NVC[h] >= (g + 1) * KG for g in range(NGRP) for h in range(GH0[g], HKV))

QBEG, QEND = 0, 39
KBEG, KEND = 39, 196
OBEG, OEND = 196, 1
LAG = 14
ELAG = 7

LAST = (2048, 2048, 2048, 1024, 512, 512)
LAST0 = 4096
NSEM = 12 + len(LAST)

f32 = jnp.float32
bf16 = jnp.bfloat16
u32 = jnp.uint32


def _mo(i, n):
    return i if isinstance(i, int) else pl.multiple_of(i, n)


def _dot(a, b):
    return jnp.dot(a, b, preferred_element_type=f32)


def _dot_nt(a, b):
    return jax.lax.dot_general(a, b, (((1,), (1,)), ((), ())), preferred_element_type=f32)


def _fold(r):
    return r[0:8] + r[8:16]


def _hilo(x):
    hi = x.astype(bf16)
    lo = (x - hi.astype(f32)).astype(bf16)
    return jnp.concatenate([hi, lo], axis=0)


def _rowsum(y):
    y = y + pltpu.roll(y, 4, 0)
    y = y + pltpu.roll(y, 2, 0)
    y = y + pltpu.roll(y, 1, 0)
    return y


def _kernel(x_hbm, k_hbm, v_hbm, wq_hbm, wo_hbm, w1_hbm, w2_hbm, o_ref,
            xbuf, k1buf, v1buf, wq, wo, w1, w2, qs, csq, cs1, x0out, pbuf, lbuf,
            qs1, wqf, wof, wqu, wou, wsm, zsm, sem):
    def heads_cp(src, b, dst, h0, n, s):
        return pltpu.make_async_copy(src.at[b, pl.ds(h0, n)], dst.at[pl.ds(h0, n)], sem.at[s])

    wqcp = pltpu.make_async_copy(wq_hbm, wq.at[:, pl.ds(0, HQ * DH)], sem.at[0])
    xcp = pltpu.make_async_copy(x_hbm, xbuf, sem.at[1])
    wocp = pltpu.make_async_copy(wo_hbm, wo.at[:, pl.ds(0, D)], sem.at[4])
    w1cp = pltpu.make_async_copy(w1_hbm, w1, sem.at[5])
    w2cp = pltpu.make_async_copy(w2_hbm, w2.at[:, pl.ds(0, D)], sem.at[6])
    k1a = heads_cp(k_hbm, 1, k1buf, 0, 4, 7)
    k1b = heads_cp(k_hbm, 1, k1buf, 4, 4, 8)
    v1a = heads_cp(v_hbm, 1, v1buf, 0, 4, 9)
    v1b = heads_cp(v_hbm, 1, v1buf, 4, 2, 10)
    v1c = heads_cp(v_hbm, 1, v1buf, 6, 1, 11)
    last_off = [(LAST0 + sum(LAST[:i])) % SK for i in range(len(LAST))]
    vlast = [pltpu.make_async_copy(v_hbm.at[1, HKV - 1, pl.ds(last_off[i], LAST[i])],
                                   v1buf.at[HKV - 1, pl.ds(last_off[i], LAST[i])], sem.at[12 + i])
             for i in range(len(LAST))]

    row8 = jax.lax.broadcasted_iota(jnp.int32, (8, T), 0)
    r8_mod = row8 % REP
    r8_lo = row8 < REP
    zero8 = jnp.zeros((8, T), f32)

    def stats(xt):
        s = (xt[0] + xt[1]) + (xt[2] + xt[3])
        m = jnp.sum(s, axis=-1, keepdims=True) * (1.0 / D)
        c = [t - m for t in xt]
        v = (c[0] * c[0] + c[1] * c[1]) + (c[2] * c[2] + c[3] * c[3])
        var = jnp.sum(v, axis=-1, keepdims=True) * (1.0 / D)
        return m, jax.lax.rsqrt(var + EPS)

    def q_head(q, h, dst):
        t = q[:, 0:DH]
        for i in range(1, REP):
            t = jnp.where(r8_mod == i, q[:, i * DH:(i + 1) * DH], t)
        a = jnp.where(r8_lo, t, 0.0)
        b = jnp.where(r8_lo, 0.0, t)
        blocks = [jnp.concatenate(p, axis=0).astype(bf16)
                  for p in ((a, zero8), (b, zero8), (zero8, a), (zero8, b))]
        dst[h] = jnp.concatenate(blocks, axis=1)

    def make_q(xt, dst):
        lc = jnp.concatenate([_hilo(t) for t in xt], axis=1)
        m, rstd = stats(xt)
        sc = rstd * SCALE
        for h in range(HKV):
            r = _fold(_dot(lc, wq[:, h * HW:(h + 1) * HW]))
            q_head((r - m * csq[:, h * HW:(h + 1) * HW]) * sc, h, dst)

    def softmax_p(s):
        mx = jnp.maximum(s[0:8], s[8:16])
        m = jnp.max(mx, axis=-1, keepdims=True)
        mb = jnp.broadcast_to(m, (8, T))
        mb = jnp.maximum(mb, pltpu.roll(mb, 4, 0))
        mb = jnp.concatenate([mb, mb], axis=0)
        p = jnp.exp(s - mb[:, :1])
        l = jnp.sum(p[0:8] + p[8:16], axis=-1, keepdims=True)
        lb = jnp.broadcast_to(l, (8, T))
        lb = lb + pltpu.roll(lb, 4, 0)
        return p.astype(bf16), lb

    def make_ocat(rs, lb):
        o = jnp.where(r8_lo, rs[0][0:8], rs[1][0:8]) + jnp.where(r8_lo, rs[2][8:16], rs[3][8:16])
        o = o / lb
        return jnp.concatenate([_hilo(jnp.where(r8_mod == i, o, 0.0)) for i in range(REP)], axis=1)

    def wo_head(ocat, h):
        return _fold(_dot(ocat, wo[pl.ds(_mo(h * HW, HW), HW), 0:D]))

    def wo_last(xt, y, ocat, h):
        out = []
        for n in range(ND):
            t = _fold(_dot(ocat, wo[h * HW:(h + 1) * HW, n * T:(n + 1) * T]))
            if y is not None:
                t = t + y[:, n * T:(n + 1) * T]
            out.append(xt[n] + _rowsum(t))
        return out

    def ffn(xt):
        lhs = [_hilo(t) for t in xt]
        m, rstd = stats(xt)
        acc = None
        for k in range(ND):
            t = _fold(_dot(lhs[k], w1[k * T:(k + 1) * T, :]))
            acc = t if acc is None else acc + t
        hh = (acc - m * cs1[...]) * rstd
        hh = hh * jax.nn.sigmoid(hh)
        hl = _hilo(hh)
        acc = None
        for k in range(NF):
            t = _fold(_dot(hl[:, k * T:(k + 1) * T], w2[k * T:(k + 1) * T, 0:D]))
            acc = t if acc is None else acc + t
        return [xt[n] + acc[:, n * T:(n + 1) * T] for n in range(ND)]

    def load_x(b):
        xin = xbuf[...].astype(f32)
        return [jnp.broadcast_to(xin[b:b + 1, n * T:(n + 1) * T], (8, T)) for n in range(ND)]

    def batch0(k0buf, v0buf):
        k0cp = pltpu.make_async_copy(k_hbm.at[0], k0buf, sem.at[2])
        v0cp = pltpu.make_async_copy(v_hbm.at[0], v0buf, sem.at[3])
        wqcp.start()
        order = [xcp, k0cp, v0cp, wocp, w1cp, w2cp, k1a, k1b, v1a, v1b, v1c] + vlast

        def issue(i, c):
            for j, cp in enumerate(order):
                @pl.when(i == j)
                def _():
                    cp.start()
            zsm[0] = i // len(order)
            return c

        jax.lax.fori_loop(0, len(order), issue, 0)

        def s_xpose(h):
            qh = qs[h]
            s = None
            for g in range(NG):
                t = _dot_nt(qh[:, g * DH:(g + 1) * DH], k0buf[h, pl.ds(g * QK, QK), :])
                s = t if s is None else s + t
            return s

        def pv0(p, h):
            return [_dot(p, v0buf[h, pl.ds(g * QK, QK), :]) for g in range(NG)]

        xcp.wait()
        wqcp.wait()
        ones16 = jnp.ones((16, D), bf16)
        csq[...] = _dot(ones16, wq[:, 0:HQ * DH])[0:8]
        x0 = load_x(0)
        make_q(x0, qs)
        make_q(load_x(1), qs1)
        wqu[:, 0:(HKV - NVQ) * HW] = pltpu.bitcast(wq[:, 0:(HKV - NVQ) * HW], u32)

        def cvt_q(j, c):
            r = pl.ds(pl.multiple_of(j * 64, 64), 64)
            for h in range(NVQ):
                hh = HKV - NVQ + h
                wqf[h, r, :] = wq[r, hh * HW:(hh + 1) * HW].astype(f32)
            return c

        jax.lax.fori_loop(0, D // 64, cvt_q, 0)

        def body00a(h, carry):
            p, lb = softmax_p(s_xpose(h))
            pbuf[h] = p
            lbuf[h] = lb
            return carry

        def body00b(h, carry):
            qs[h] = make_ocat(pv0(pbuf[h], h), lbuf[h])
            return carry

        k0cp.wait()
        jax.lax.fori_loop(0, HKV, body00a, 0)
        v0cp.wait()
        jax.lax.fori_loop(0, HKV, body00b, 0)
        wocp.wait()
        y = None
        for h in range(HKV - 1):
            t = wo_head(qs[h], h)
            y = t if y is None else y + t
        x0 = wo_last(x0, y, qs[HKV - 1], HKV - 1)
        wou[:, 0:D] = pltpu.bitcast(wo[(HKV - 2) * HW:HKV * HW, 0:D], u32)
        for hh in range(HKV):
            wsum = _dot_nt(jnp.ones((16, D), bf16), wo[hh * HW:(hh + 1) * HW, 0:D])[0:8]
            t = wsum[:, 0:DH]
            for i in range(1, REP):
                t = jnp.where(r8_mod == i, wsum[:, i * DH:(i + 1) * DH], t)
            wsm[hh * 8:(hh + 1) * 8, :] = t

        def cvt_o(j, c):
            r = pl.ds(pl.multiple_of(j * 64, 64), 64)
            for h in range(NVO):
                wof[h, r, :] = wo[pl.ds(pl.multiple_of(h * HW + j * 64, 64), 64), 0:D].astype(f32)
            return c

        jax.lax.fori_loop(0, HW // 64, cvt_o, 0)
        w1cp.wait()
        w2cp.wait()
        cs1[...] = _dot(ones16, w1[...])[0:8]
        x0 = ffn(x0)
        make_q(x0, qs)

        def body01(h, y):
            p, lb = softmax_p(s_xpose(h))
            return y + wo_head(make_ocat(pv0(p, h), lb), h)

        y = jax.lax.fori_loop(0, HKV, body01, jnp.zeros((8, D), f32))
        y = _rowsum(y)
        x0 = [x0[n] + y[:, n * T:(n + 1) * T] for n in range(ND)]
        x0 = ffn(x0)
        x0out[...] = jnp.concatenate(x0, axis=1)

    pl.run_scoped(batch0, pltpu.VMEM((HKV, SK, DH), bf16), pltpu.VMEM((HKV, SK, DH), bf16))

    def batch1(ktu, v1u, w1u, w2u, w1t, w2s, w2f, ktf, ktmp, cmask, cmask2, *bufs):
        sbufs = bufs[:HKV]
        svs = bufs[HKV:2 * HKV]
        qrb = bufs[2 * HKV:]

        zero = zsm[0]
        zvec = jnp.full((8, T), zero, jnp.int32)

        def tie1(a, dep):
            return pltpu.bitcast(pltpu.bitcast(a, jnp.int32) | (pltpu.bitcast(dep, jnp.int32) & zvec), f32)

        cmask[pl.ds(pl.multiple_of(zero, T), T), :] = jnp.where(
            jax.lax.broadcasted_iota(jnp.int32, (T, T), 0) == jax.lax.broadcasted_iota(jnp.int32, (T, T), 1), -1, 0)

        r512 = jax.lax.broadcasted_iota(jnp.int32, (4 * DH, T), 0)
        cmask2[pl.ds(pl.multiple_of(zero, T), 4 * DH), :] = jnp.where(
            jax.lax.broadcasted_iota(jnp.int32, (4 * DH, T), 1) == 2 * (r512 >> 3) + ((r512 >> 1) & 1), -1, 0)

        def colm(rowv, msk):
            d = pltpu.bitcast(pltpu.bitcast(rowv, jnp.int32) & msk, f32)
            return jnp.broadcast_to(jnp.sum(d, axis=-1, keepdims=True), (8, T))

        def colb(rowv, j):
            return colm(rowv, cmask[8 * j:8 * j + 8, :])

        x1 = load_x(1)
        eye = (jax.lax.broadcasted_iota(jnp.int32, (DH, DH), 0)
               == jax.lax.broadcasted_iota(jnp.int32, (DH, DH), 1)).astype(bf16)

        w1u[...] = pltpu.bitcast(w1[:, 0:NM1 * T], u32)
        w2u[:, 0:D] = pltpu.bitcast(w2[FA * T:, 0:D], u32)
        w2f[...] = w2[0:(FA + FXM) * T, 0:D].astype(f32)
        w1t[...] = w1[:, NM1 * T:].astype(f32)

        w2s[...] = _dot_nt(jnp.ones((16, D), bf16), w2[:, 0:D])[0:8]

        orows = {}

        def o_norm(o, lb):
            o = o * (1.0 / lb)
            ocat = jnp.concatenate([jnp.where(r8_mod == i, o, 0.0).astype(bf16) for i in range(REP)], axis=1)
            return o.astype(bf16).astype(f32), ocat

        def wo_last_m(xt, y, rs, lb, prev=None):
            pre = jnp.where(row8 == 0, (xt[0] + xt[1]) + (xt[2] + xt[3]), 0.0)
            if prev is None:
                pre = pre + ((y[:, 0:T] + y[:, T:2 * T]) + (y[:, 2 * T:3 * T] + y[:, 3 * T:4 * T]))
            else:
                e = None
                for h in range(NVO):
                    t = orows[h] * wsm[h * 8:(h + 1) * 8, :]
                    e = t if e is None else e + t
                pre = pre + e * 0.5 + prev[0] * wsm[(HKV - 2) * 8:(HKV - 1) * 8, :]
                y = _dot(prev[1], pltpu.bitcast(wou[0:HW // 2, 0:D], bf16)) + y
            o, ocat = o_norm(rs, lb)
            m = jnp.sum(_rowsum(o * wsm[(HKV - 1) * 8:HKV * 8, :] + pre), axis=-1, keepdims=True) * (1.0 / D)
            out = []
            for n in range(ND):
                t = _dot(ocat, pltpu.bitcast(wou[HW // 2:HW, n * T:(n + 1) * T], bf16)) + y[:, n * T:(n + 1) * T]
                out.append(xt[n] + _rowsum(t))
            return out, m

        def rstd_of(c):
            v = (c[0] * c[0] + c[1] * c[1]) + (c[2] * c[2] + c[3] * c[3])
            return jax.lax.rsqrt(jnp.sum(v, axis=-1, keepdims=True) * (1.0 / D) + EPS)

        def ffn_split(xt, m, ntail, fx):
            xc = [t - m for t in xt]
            lhs = [t.astype(bf16) for t in xc]
            rh = rstd_of(xc) * 0.5

            def act(a):
                z = a * rh
                return z * jnp.tanh(z) + z

            acc = None
            for k in range(ND):
                t = _dot(lhs[k], pltpu.bitcast(w1u[k * (T // 2):(k + 1) * (T // 2), 0:FA * T], bf16))
                acc = t if acc is None else t + acc
            ha = act(acc)
            lc = jnp.concatenate(lhs, axis=1)
            hm = []
            for n in range(FA, NM1):
                t = act(_dot(lc, pltpu.bitcast(w1u[:, n * T:(n + 1) * T], bf16)))
                if n - FA < fx:
                    ha = jnp.concatenate([ha, t], axis=1)
                    hm.append(None)
                else:
                    hm.append(t.astype(bf16))
            accs = [None, None]
            for kg in range(D // 8):
                c = colb(xc[kg // 16], kg % 16)
                t = w1t[kg * 8:(kg + 1) * 8, :] * jnp.concatenate([c] * FC, axis=1)
                accs[kg % 2] = t if accs[kg % 2] is None else accs[kg % 2] + t
            hc = act(_rowsum(accs[0] + accs[1])).astype(bf16)
            hm += [hc[:, n * T:(n + 1) * T] for n in range(FC)]
            accs = [None, None]
            for g in range((FA + fx) * T // 8):
                c = colb(ha[:, (g // 16) * T:(g // 16 + 1) * T], g % 16)
                t = w2f[g * 8:(g + 1) * 8, :] * jnp.concatenate([c] * ND, axis=1)
                accs[g % 2] = t if accs[g % 2] is None else accs[g % 2] + t
            yv = _rowsum(accs[0] + accs[1])
            order = list(range(fx, NM2))
            nk = len(order) - ntail
            acc = None
            for k in order[:nk]:
                t = _dot(hm[k], pltpu.bitcast(w2u[k * (T // 2):(k + 1) * (T // 2), 0:D], bf16))
                acc = t if acc is None else t + acc
            out = []
            for n in range(ND):
                t = xt[n] + (acc[:, n * T:(n + 1) * T] + yv[:, n * T:(n + 1) * T])
                if ntail:
                    lt = jnp.concatenate([hm[k] for k in order[nk:]], axis=1)
                    wt = jnp.concatenate([pltpu.bitcast(w2u[k * (T // 2):(k + 1) * (T // 2), n * T:(n + 1) * T], bf16)
                                          for k in order[nk:]], axis=0)
                    t = _dot(lt, wt) + t
                out.append(t)
            e = None
            for n in range(NF):
                hn = ha[:, n * T:(n + 1) * T] if n < FA + fx else hm[n - FA].astype(f32)
                t = hn * w2s[:, n * T:(n + 1) * T]
                e = t if e is None else e + t
            e = e + ((xt[0] + xt[1]) + (xt[2] + xt[3]))
            return out, jnp.sum(e, axis=-1, keepdims=True) * (1.0 / D)

        def s_xpose_t(h):
            qh = qs1[h]
            s = None
            for g in range(NG):
                lhs = jnp.concatenate([qh[:, g * DH:(g + 1) * DH], eye], axis=0)
                t = _dot_nt(lhs, k1buf[h, pl.ds(g * QK, QK), :])
                ktu[h, pl.ds(g * (DH // 2), DH // 2), 0:QK] = pltpu.bitcast(t[16:].astype(bf16), u32)
                if g >= 2:
                    ktmp[pl.ds((g - 2) * DH, DH), 0:NVCM * T] = t[16:, 0:NVCM * T]
                s = t[:16] if s is None else s + t[:16]
            return s

        def k_operand(h):
            roww = jax.lax.broadcasted_iota(jnp.int32, (8, KG * T), 0)
            for g in range(NGRP):
                @pl.when(h >= GH0[g])
                def _():
                    def blk(j, c):
                        a = ktmp[pl.ds(pl.multiple_of(j * 8, 8), 8), g * KG * T:(g + 1) * KG * T]
                        b = ktmp[pl.ds(pl.multiple_of(DH + j * 8, 8), 8), g * KG * T:(g + 1) * KG * T]
                        for k in range(4):
                            idx = 2 * k + ((roww >> 1) & 1)
                            ktf[GBASE[g] + h - GH0[g], pl.ds(pl.multiple_of(j * 32 + k * 8, 8), 8), 0:KG * T] = jnp.where(
                                roww < 4, jnp.take_along_axis(a, idx, axis=0), jnp.take_along_axis(b, idx, axis=0))
                        return c

                    jax.lax.fori_loop(0, DH // 8, blk, 0, unroll=4)

        def pv_copy(p, h, off, n):
            v = v1buf[h, pl.ds(off, n), :]
            v1u[h, pl.ds(off // 2, n // 2), :] = pltpu.bitcast(v, u32)
            return _dot(p, v)

        def body10a(h, carry):
            @pl.when(h == 0)
            def _():
                k1a.wait()

            @pl.when(h == 4)
            def _():
                k1b.wait()

            p, lb = softmax_p(s_xpose_t(h))
            pbuf[h] = p
            lbuf[h] = lb
            k_operand(h)
            return carry

        def body10b(h, y):
            for hh, cp in ((0, v1a), (4, v1b), (6, v1c)):
                @pl.when(h == hh)
                def _():
                    cp.wait()

            p = pbuf[h]
            rs = [pv_copy(p, h, g * QK, QK) for g in range(NG)]
            return y + wo_head(make_ocat(rs, lbuf[h]), h)

        jax.lax.fori_loop(0, HKV, body10a, 0)
        y = jax.lax.fori_loop(0, HKV - 1, body10b, jnp.zeros((8, D), f32))
        h = HKV - 1
        p = pbuf[h]
        lb = lbuf[h]
        rs = [None] * NG
        for i in range(len(LAST)):
            vlast[i].wait()
            g = last_off[i] // QK
            c0 = last_off[i] - g * QK
            t = pv_copy(p[:, c0:c0 + LAST[i]], h, last_off[i], LAST[i])
            rs[g] = t if rs[g] is None else t + rs[g]
        o8 = jnp.where(r8_lo, rs[0][0:8], rs[1][0:8]) + jnp.where(r8_lo, rs[2][8:16], rs[3][8:16])
        x1, m = wo_last_m(x1, y, o8, lb)
        x1, m = ffn_split(x1, m, 4, FX[0])

        def q_head2(q, h):
            if h > 0:
                q = q * sc8
            t = q[:, 0:DH]
            for i in range(1, REP):
                t = jnp.where(r8_mod == i, q[:, i * DH:(i + 1) * DH], t)
            ab = jnp.concatenate([jnp.where(r8_lo, t, 0.0), jnp.where(r8_lo, 0.0, t)], axis=1)
            qs[h, :, 0:2 * DH] = jnp.concatenate([ab, ab], axis=0).astype(bf16)
            if NVC[h]:
                qr = q.astype(bf16).astype(f32)
                odd = (row8 & 1) == 1
                qrb[h][pl.ds(pl.multiple_of(zero, 8), 8), :] = jnp.concatenate(
                    [jnp.where(odd, qr[:, (2 * a + 1) * DH:(2 * a + 2) * DH], qr[:, 2 * a * DH:(2 * a + 1) * DH])
                     for a in range(2)], axis=1)

        xc = [t - m for t in x1]
        lhs = [t.astype(bf16) for t in xc]
        rstd = rstd_of(xc)
        sc8 = rstd * (SCALE * LOG2E)
        sc = jnp.concatenate([sc8, sc8], axis=0)
        b1 = (row8 & 2) == 0

        row16 = pl.ds(pl.multiple_of(zero, 16), 16)
        row_lo = pl.ds(pl.multiple_of(zero, 8), 8)

        def tie_b(a, dep):
            return pltpu.bitcast(pltpu.bitcast(a, jnp.int32) | (pltpu.bitcast(dep, jnp.int32) & zvec), bf16)

        def or_all(vals):
            bits = [pltpu.bitcast(a, jnp.int32) for a in vals]
            while len(bits) > 1:
                bits = [bits[k] | bits[k + 1] if k + 1 < len(bits) else bits[k] for k in range(0, len(bits), 2)]
            return pltpu.bitcast(bits[0], f32)

        gstep = [0]
        deps = {}
        events = {}

        def pre_step(a):
            for d in deps.pop(gstep[0], ()):
                a = tie_b(a, d)
            return a

        toks = []

        def post_step(tok):
            toks.append(tok)
            for task, dl in events.pop(gstep[0], ()):
                mark = task.send(tok)
                if mark is not None:
                    deps.setdefault(dl, []).append(mark)
            gstep[0] += 1

        mv = {}

        def k_task(h):
            mark = None
            mx = None
            for g in range(NVC[h] // KG):
                acc = [None, None]
                for dp in range(DH // 2):
                    tok = yield mark
                    mark = None
                    qr = qrb[h][...]
                    msk = cmask2[8 * dp:8 * dp + 8, :]
                    ktr = ktf[GBASE[g] + h - GH0[g], dp * 8:dp * 8 + 8, 0:KG * T]
                    for a in range(2):
                        qd = colm(tie1(qr[:, a * DH:(a + 1) * DH], tok), msk)
                        pr = ktr * jnp.concatenate([qd] * KG, axis=1)
                        acc[a] = pr if acc[a] is None else acc[a] + pr
                mark = or_all([acc[a][:, c * T:(c + 1) * T] for c in range(KG) for a in range(2)])
                st = jnp.where(jnp.concatenate([b1] * KG, axis=1),
                               acc[0] + pltpu.roll(acc[0], 6, 0), acc[1] + pltpu.roll(acc[1], 2, 0))
                svs[h][row_lo, g * KG * T:(g + 1) * KG * T] = st
                for c in range(KG):
                    t = st[:, c * T:(c + 1) * T]
                    mx = t if mx is None else jnp.maximum(mx, t)
            mv[h] = mx
            yield mx

        def q_task():
            mark = None
            for h0 in range(HKV - NVQ, HKV, 2):
                acc = [None, None]
                for kg in range(D // 8):
                    tok = yield mark
                    mark = None
                    c4 = jnp.concatenate([colb(tie1(xc[kg // 16], tok), kg % 16)] * 4, axis=1)
                    for a in range(2):
                        t = wqf[h0 + a - (HKV - NVQ), kg * 8:(kg + 1) * 8, :] * c4
                        acc[a] = t if acc[a] is None else acc[a] + t
                qq = [_rowsum(acc[a]) for a in range(2)]
                for a in range(2):
                    q_head2(qq[a], h0 + a)
                mark = or_all([qq[a][:, n * T:(n + 1) * T] for a in range(2) for n in range(ND)])
            yield mark

        yacc = [None]

        def o_task():
            mark = None
            for h in range(NVO):
                for kg in range(HW // 8):
                    tok = yield mark
                    mark = None
                    i = kg // 16
                    c = colb(tie1(jnp.broadcast_to(orows[h][i:i + 1, :], (8, T)), tok), kg % 16)
                    t = wof[h, kg * 8:(kg + 1) * 8, :] * jnp.concatenate([c] * 4, axis=1)
                    yacc[0] = t if yacc[0] is None else yacc[0] + t
                mark = or_all([yacc[0][:, n * T:(n + 1) * T] for n in range(ND)])
            yield mark

        def qk(h):
            qh = qs[h, :, 0:2 * DH]
            nv = NVC[h]
            mx = None

            def lhs():
                return jnp.concatenate([pre_step(qh[:, 0:DH]), qh[:, DH:2 * DH]], axis=1)

            for c in range(0, nv, 2):
                w = min(2, nv - c)
                st = _dot(lhs(), pltpu.bitcast(ktu[h, 0:DH, c * T:(c + w) * T], bf16))[0:8]
                sbufs[h][row_lo, c * T:(c + w) * T] = st
                for cc in range(w):
                    t = st[:, cc * T:(cc + 1) * T]
                    mx = t if mx is None else jnp.maximum(mx, t)
                post_step(st[:, 0:T])
            for c in range(nv, NC):
                kk = jnp.concatenate([pltpu.bitcast(ktu[h, 0:DH, c * T:(c + 1) * T], bf16),
                                      pltpu.bitcast(ktu[h, DH:2 * DH, c * T:(c + 1) * T], bf16)], axis=1)
                st = _dot(lhs(), kk)[0:8]
                sbufs[h][row16, c * T:(c + 1) * T] = jnp.concatenate([st[:, 0:T], st[:, T:2 * T]], axis=0)
                t = jnp.maximum(st[:, 0:T], st[:, T:2 * T])
                mx = t if mx is None else jnp.maximum(mx, t)
                post_step(st[:, 0:T])
            return mx

        def pv(mx, h):
            if NVC[h]:
                mx = jnp.maximum(mx, mv.pop(h))
            mb = jnp.broadcast_to(jnp.max(mx, axis=-1, keepdims=True), (8, T))
            mb8 = jnp.maximum(mb, pltpu.roll(mb, 4, 0))
            acc = None
            ls = None
            for c in range(NC):
                if c < NVC[h]:
                    sv = jnp.concatenate([sbufs[h][0:8, c * T:(c + 1) * T], svs[h][:, c * T:(c + 1) * T]], axis=0)
                else:
                    sv = sbufs[h][:, c * T:(c + 1) * T]
                mbc = tie1(mb8, toks[gstep[0] - ELAG])
                e = sv - jnp.concatenate([mbc, mbc], axis=0)
                p = jnp.exp2(e * sc if h == 0 else e)
                t = p[0:8] + p[8:16]
                ls = t if ls is None else ls + t
                vv = jnp.concatenate(
                    [pltpu.bitcast(v1u[h, pl.ds((g * QK + c * T) // 2, T // 2), :], bf16) for g in range(NG)], axis=1)
                r = _dot(pre_step(p.astype(bf16)), vv)
                t = (jnp.where(r8_lo, r[0:8, 0:T], r[0:8, T:2 * T])
                     + jnp.where(r8_lo, r[8:16, 2 * T:3 * T], r[8:16, 3 * T:4 * T]))
                acc = t if acc is None else acc + t
                post_step(r[0:8, 0:T])
            lb = jnp.broadcast_to(jnp.sum(ls, axis=-1, keepdims=True), (8, T))
            lb = lb + pltpu.roll(lb, 4, 0)
            return acc, lb

        nsteps = 4 * (HKV - NVQ) + sum(NC + NC - nv + (nv + 1) // 2 for nv in NVC)

        def spread(task, n, beg, width):
            next(task)
            for j in range(n):
                rel = int(beg + width * j / n)
                events.setdefault(rel, []).append((task, rel + LAG))

        pos = 0.0
        for h in range(HKV):
            if NVC[h]:
                w = (KEND - KBEG) * NVC[h] / sum(NVC)
                spread(k_task(h), NVC[h] // KG * (DH // 2), KBEG + pos, w)
                pos += w
        spread(o_task(), NVO * (HW // 8), OBEG, nsteps - OEND - OBEG)
        spread(q_task(), NVQ // 2 * (D // 8), QBEG, QEND - QBEG)

        acc = None
        for k in range(ND):
            t = _dot(lhs[k], pltpu.bitcast(wqu[k * (T // 2):(k + 1) * (T // 2), 0:HW], bf16))
            post_step(t[:, 0:T])
            acc = t if acc is None else acc + t
        q_head2(acc, 0)
        lc = jnp.concatenate(lhs, axis=1)
        for h in range(1, HKV - NVQ):
            parts = []
            for n in range(ND):
                parts.append(_dot(lc, pltpu.bitcast(wqu[:, h * HW + n * T:h * HW + (n + 1) * T], bf16)))
                post_step(parts[-1])
            q_head2(jnp.concatenate(parts, axis=1), h)
        ms = {0: qk(0)}
        prev = None
        for h in range(HKV):
            if h + 1 < HKV:
                ms[h + 1] = qk(h + 1)
            rs, lb = pv(ms.pop(h), h)
            if h < NVO:
                orows[h] = (rs + pltpu.roll(rs, 4, 0)) / lb
            elif h < HKV - 1:
                prev = o_norm(rs, lb)
        assert not events, sorted(events)
        x1, m = wo_last_m(x1, yacc[0], rs, lb, prev)
        x1, _ = ffn_split(x1, m, 0, FX[1])
        row2 = jax.lax.broadcasted_iota(jnp.int32, (2, D), 0)
        xo1 = jnp.concatenate(x1, axis=1)
        o_ref[...] = jnp.where(row2 == 0, x0out[0:2, :], xo1[0:2, :]).astype(o_ref.dtype)

    pl.run_scoped(batch1,
                  pltpu.VMEM((HKV, NG * DH // 2, QK + PAD), u32),
                  pltpu.VMEM((HKV, SK // 2, DH), u32),
                  pltpu.VMEM((D // 2, NM1 * T), u32),
                  pltpu.VMEM((NM2 * T // 2, D + PAD), u32),
                  pltpu.VMEM((D, FC * T), f32),
                  pltpu.VMEM((8, F), f32),
                  pltpu.VMEM(((FA + FXM) * T, D), f32),
                  pltpu.VMEM((NSLOT, 4 * DH, KG * T + PAD), f32),
                  pltpu.VMEM((2 * DH, NVCM * T + PAD), f32),
                  pltpu.VMEM((T, T), jnp.int32),
                  pltpu.VMEM((4 * DH, T), jnp.int32),
                  *[pltpu.VMEM((16, QK), f32) for _ in range(HKV)],
                  *[pltpu.VMEM((8, NVCM * T), f32) for _ in range(HKV)],
                  *[pltpu.VMEM((8, 2 * DH), f32) for _ in range(HKV)])


def _compiler_params():
    vmem = 120 * 1024 * 1024
    try:
        return pltpu.CompilerParams(vmem_limit_bytes=vmem, disable_semaphore_checks=True)
    except TypeError:
        return pltpu.CompilerParams(vmem_limit_bytes=vmem)


@jax.jit
def pallas_interleave_layers__gqa_block_cached__dense_activation_silu__decode_kernel(
    A_x, A_k_cache, A_v_cache, A_wq, A_wo, B_x, B_w1, B_w2,
):
    del B_x
    any_spec = pl.BlockSpec(memory_space=pl.ANY)
    return pl.pallas_call(
        _kernel,
        out_shape=jax.ShapeDtypeStruct((B, D), A_x.dtype),
        in_specs=[any_spec] * 7,
        out_specs=pl.BlockSpec(memory_space=pltpu.VMEM),
        scratch_shapes=[
            pltpu.VMEM((B, D), bf16),
            pltpu.VMEM((HKV, SK, DH), bf16),
            pltpu.VMEM((HKV, SK, DH), bf16),
            pltpu.VMEM((D, HQ * DH + PAD), bf16),
            pltpu.VMEM((HQ * DH, D + PAD), bf16),
            pltpu.VMEM((D, F), bf16),
            pltpu.VMEM((F, D + PAD), bf16),
            pltpu.VMEM((HKV, 16, NG * DH), bf16),
            pltpu.VMEM((8, HQ * DH), f32),
            pltpu.VMEM((8, F), f32),
            pltpu.VMEM((8, D), f32),
            pltpu.VMEM((HKV, 16, QK), bf16),
            pltpu.VMEM((HKV, 8, T), f32),
            pltpu.VMEM((HKV, 16, NG * DH), bf16),
            pltpu.VMEM((NVQ, D, HW), f32),
            pltpu.VMEM((NVO, HW, D), f32),
            pltpu.VMEM((D // 2, (HKV - NVQ) * HW + PAD), u32),
            pltpu.VMEM((HW, D + PAD), u32),
            pltpu.VMEM((HKV * 8, T), f32),
            pltpu.SMEM((1,), jnp.int32),
            pltpu.SemaphoreType.DMA((NSEM,)),
        ],
        compiler_params=_compiler_params(),
    )(A_x.reshape(B, D), A_k_cache, A_v_cache, A_wq, A_wo, B_w1, B_w2).reshape(A_x.shape)
```
